```python
import os as _os
_os.environ.setdefault("JAX_PLATFORMS", "cpu")
import jax
import jax.numpy as jnp

def _softmax(x, axis=-1):
    return jax.nn.softmax(x, axis=axis)
def _gelu(x):
    return jax.nn.gelu(x, approximate=True)
def _silu(x):
    return jax.nn.silu(x)
def _sigmoid(x):
    return jax.nn.sigmoid(x)
def _layernorm(x, axis=-1, eps=1e-5):
    m = jnp.mean(x, axis=axis, keepdims=True)
    v = jnp.var(x, axis=axis, keepdims=True)
    return (x - m) / jnp.sqrt(v + eps)
def _scatter_add(tgt, idx, src, axis=0):
    return tgt.at[idx].add(src)
def _segment_sum(src, seg, n):
    return jax.ops.segment_sum(src, seg, n)
class _Rng:
    def __init__(self, key):
        self._k = key
    def _next(self):
        self._k, sub = jax.random.split(self._k)
        return sub
    def normal(self, shape):
        return jax.random.normal(self._next(), shape, dtype=jnp.bfloat16)
    def randint(self, lo, hi, shape):
        return jax.random.randint(self._next(), shape, lo, hi, dtype=jnp.int32)
    def uniform(self, shape, lo=0.0, hi=1.0):
        return jax.random.uniform(self._next(), shape, jnp.bfloat16, lo, hi)
    def permutation(self, n):
        return jax.random.permutation(self._next(), n)


kernel_name = 'standalone__channel_attn_cbam__vision'

def setup_inputs():
    _rng = _Rng(jax.random.key(int.from_bytes(__import__("os").urandom(4), "little")))
    _w = (lambda a: (lambda t: t.astype(jnp.bfloat16) if jnp.issubdtype(t.dtype, jnp.floating) else t)(jnp.asarray(a)))
    H = W = 384
    C = 192
    r = max(C // 4, 1)
    return {
        "x": _w((lambda *s: _rng.normal(s) * 0.2)(1, H, W, C) + (lambda *s: _rng.normal(s) * 0.2)(1, 1, 1, C) * 2.0),
        "w1": _w((lambda *s: _rng.normal(s) * 0.2)(C, r)),
        "w2": _w((lambda *s: _rng.normal(s) * 0.2)(r, C)),
    }

def reference(x, w1, w2):
    B, H, W, C = x.shape
    xf = x.reshape(B, H * W, C)
    gap = jnp.mean(xf, 1)
    gmp = jnp.amax(xf, 1)
    h_a = gap @ w1
    h_a = h_a * (lambda x, dt: x.astype(dt))(h_a > 0, h_a.dtype)
    h_m = gmp @ w1
    h_m = h_m * (lambda x, dt: x.astype(dt))(h_m > 0, h_m.dtype)
    scale = _sigmoid(h_a @ w2 + h_m @ w2)
    return x * scale[:, None, None, :]
```

```python
import functools

import jax
import jax.numpy as jnp
import jax.experimental.pallas as pl
import jax.experimental.pallas.tpu as pltpu

_H, _W, _C, _R = 384, 384, 192, 48
_LANES = 128
_WB = _W // _LANES
_CB = _C // 8
_S = 6
_HH = _H // _S
_Q = 4
_CBQ = _CB // _Q
_PR = _CBQ * _WB * 8
_NJ = _HH * _Q
_NSEM = 3

_CHUNKS = [(0, 2, 0, 64), (2, 2, 0, 64), (4, 1, 0, 64)]
_hh0 = 0
for _n in (24, 16, 10, 6, 4, 2, 1, 1):
    _CHUNKS.append((5, 1, _hh0, _n))
    _hh0 += _n
assert _hh0 == _HH


def _kernel(x_hbm, w1t_hbm, w2_hbm, o_hbm, buf, w1t_v, w2_v, w2t_v,
            acc_s, acc_m, scale, sems):
    def rd(i):
        s0, ns, h0, nh = _CHUNKS[i]
        sl = (pl.ds(s0, ns), pl.ds(h0 * _Q, nh * _Q))
        return pltpu.make_async_copy(x_hbm.at[sl], buf.at[sl], sems.at[i % _NSEM])

    w1_cp = pltpu.make_async_copy(w1t_hbm, w1t_v, sems.at[0])
    w2_cp = pltpu.make_async_copy(w2_hbm, w2_v, sems.at[0])

    rd(0).start()
    w1_cp.start()
    w2_cp.start()
    for i in range(1, _NSEM):
        rd(i).start()

    acc_s[...] = jnp.zeros(acc_s.shape, jnp.float32)
    acc_m[...] = jnp.full(acc_m.shape, -jnp.inf, jnp.float32)

    def reduce_rows(s, hh, g):
        for q in range(_Q):
            a_s = acc_s[pl.ds(q * _CBQ, _CBQ)]
            a_m = acc_m[pl.ds(q * _CBQ, _CBQ)]
            for r in range(g):
                v = buf[s, (hh + r) * _Q + q].astype(jnp.float32)
                v = v.reshape(_CBQ, _WB, 8, _LANES)
                for wb in range(_WB):
                    a_s = a_s + v[:, wb]
                    a_m = jnp.maximum(a_m, v[:, wb])
            acc_s[pl.ds(q * _CBQ, _CBQ)] = a_s
            acc_m[pl.ds(q * _CBQ, _CBQ)] = a_m

    for i, (s0, ns, h0, nh) in enumerate(_CHUNKS):
        rd(i).wait()
        if i == 0:
            w1_cp.wait()
            w2_cp.wait()
        if i + _NSEM < len(_CHUNKS):
            rd(i + _NSEM).start()
        if i == 0:
            w2t = w2_v[...].astype(jnp.float32).T
            w2t_v[...] = jnp.concatenate([w2t, w2t], axis=1).astype(jnp.bfloat16)
        g = 2 if nh % 2 == 0 else 1
        steps = nh // g

        def body(t, carry, s0=s0, h0=h0, g=g, steps=steps):
            reduce_rows(s0 + t // steps, h0 + (t % steps) * g, g)
            return carry

        if ns * steps == 1:
            reduce_rows(s0, h0, g)
        else:
            jax.lax.fori_loop(0, ns * steps, body, 0)

    ssum = jnp.sum(acc_s[...].reshape(_C, _LANES), axis=1, keepdims=True)
    smax = jnp.max(acc_m[...].reshape(_C, _LANES), axis=1, keepdims=True)
    gap = (ssum * (1.0 / (_H * _W))).astype(jnp.bfloat16)
    gmp = smax.astype(jnp.bfloat16)
    p = jnp.concatenate([jnp.broadcast_to(gap, (_C, _LANES)),
                         jnp.broadcast_to(gmp, (_C, _LANES))], axis=1)
    h = jnp.dot(w1t_v[...], p, preferred_element_type=jnp.float32)
    h = jnp.maximum(h, 0.0).astype(jnp.bfloat16)
    h2 = jnp.concatenate([h[:, :_LANES], h[:, _LANES:]], axis=0)
    z = jnp.dot(w2t_v[...], h2, preferred_element_type=jnp.float32)
    sc = jax.nn.sigmoid(z).astype(jnp.bfloat16).astype(jnp.float32)
    scale[...] = sc.reshape(_CB, 8, _LANES)

    def wr_body(j, carry):
        q = j % _Q
        sq = scale[pl.ds(q * _CBQ, _CBQ)]
        for s in range(_S):
            v = buf[s, j].astype(jnp.float32).reshape(_CBQ, _WB, 8, _LANES)
            v = v * sq[:, None]
            buf[s, j] = v.reshape(_PR, _LANES).astype(jnp.bfloat16)
        pltpu.make_async_copy(buf.at[:, j], o_hbm.at[:, j], sems.at[0]).start()
        return carry

    jax.lax.fori_loop(0, _NJ, wr_body, 0)
    pltpu.make_async_copy(buf, o_hbm, sems.at[0]).wait()


@jax.jit
def pallas_standalone__channel_attn_cbam__vision_kernel(
    x: jax.Array,
    w1: jax.Array,
    w2: jax.Array,
):
    xv = jnp.transpose(x, (0, 1, 3, 2)).reshape(_H, _CB, 8, _WB, _LANES)
    xv = jnp.transpose(xv, (0, 1, 3, 2, 4)).reshape(_S, _NJ, _PR, _LANES)
    out = pl.pallas_call(
        _kernel,
        out_shape=jax.ShapeDtypeStruct((_S, _NJ, _PR, _LANES), x.dtype),
        in_specs=[pl.BlockSpec(memory_space=pl.ANY)] * 3,
        out_specs=pl.BlockSpec(memory_space=pl.ANY),
        scratch_shapes=[
            pltpu.VMEM((_S, _NJ, _PR, _LANES), jnp.bfloat16),
            pltpu.VMEM((_R, _C), jnp.bfloat16),
            pltpu.VMEM((_R, _C), jnp.bfloat16),
            pltpu.VMEM((_C, 2 * _R), jnp.bfloat16),
            pltpu.VMEM((_CB, 8, _LANES), jnp.float32),
            pltpu.VMEM((_CB, 8, _LANES), jnp.float32),
            pltpu.VMEM((_CB, 8, _LANES), jnp.float32),
            pltpu.SemaphoreType.DMA((_NSEM,)),
        ],
        compiler_params=pltpu.CompilerParams(vmem_limit_bytes=100 * 1024 * 1024),
    )(xv, w1.T, w2)
    out = out.reshape(_H, _CB, _WB, 8, _LANES)
    out = jnp.transpose(out, (0, 1, 3, 2, 4)).reshape(1, _H, _C, _W)
    return jnp.transpose(out, (0, 1, 3, 2))
```

```python
import functools
import jax
import jax.numpy as jnp
from jax import lax
import jax.experimental.pallas as pl
import jax.experimental.pallas.tpu as pltpu

H, W, C, R = 384, 384, 192, 48
L = 128
WB = 3
CB = 24
PA, PJ, PR = 54, 64, 64
NS = 6
TPP = PR // 8
PER = CB * WB
NPH = PER // TPP
TAB = (PER - TPP + NS * TPP + 2) // WB + 1
RJ = 256
RS = 18
NG = PA // RS
SUB = RJ // PJ


def make_kernel(name='k', n0=4, depth=12, peel=1, rnd=True, split1=True, order='wi', nsem=16, mode='chunk'):
    nch = NG * RJ
    assert depth % SUB == 0 and depth < nsem + (order == 'wi')

    def kernel(x_hbm, w1t_hbm, w2_hbm, o_hbm, buf, w1t_v, w2_v, w1d, w2d, acc_s, acc_m, tab, sems, wsem):
        def slot(i):
            return sems.at[i % nsem if isinstance(i, int) else i & (nsem - 1)]

        def rd_start(i):
            if isinstance(i, int):
                a0, j = (i // RJ) * RS, i % RJ
            else:
                a0, j = lax.shift_right_logical(i, 8) * RS, i & (RJ - 1)
            for t, (o, n) in enumerate(((0, n0), (n0, RS - n0))):
                sl = (pl.ds(a0 + o, n), j)
                pltpu.make_async_copy(x_hbm.at[sl], buf.at[sl], slot(i)).start(priority=t)

        def rd_wait(i):
            sl = (pl.ds(0, RS), 0)
            pltpu.make_async_copy(x_hbm.at[sl], buf.at[sl], slot(i)).wait()

        w1_cp = pltpu.make_async_copy(w1t_hbm, w1t_v, wsem)
        w2_cp = pltpu.make_async_copy(w2_hbm, w2_v, wsem)
        for i in range(depth):
            rd_start(i)
        w1_cp.start()
        w2_cp.start()

        acc_s[...] = jnp.zeros(acc_s.shape, jnp.float32)
        acc_m[...] = jnp.full(acc_m.shape, -jnp.inf, jnp.float32)

        def dup_t(w_ref):
            w = w_ref[...].astype(jnp.float32)
            z16 = jnp.zeros((64 - R, C), jnp.float32)
            return jnp.concatenate([w, z16, w, z16], axis=0).T.reshape(CB, 8, L)

        def reduce_col(blk, j, c, acc):
            for ph in range(NPH):
                u = buf[blk[ph], j].astype(jnp.float32)
                v = buf[blk[ph] + NPH, j].astype(jnp.float32)
                s = u + v
                m = jnp.maximum(u, v)
                for hf in range(2):
                    cb = (ph * TPP + 2 * c + hf) // WB
                    if cb not in acc:
                        acc[cb] = (acc_s[cb], acc_m[cb])
                    a, b = acc[cb]
                    acc[cb] = (a + s[hf * 8:hf * 8 + 8], jnp.maximum(b, m[hf * 8:hf * 8 + 8]))

        def flush(acc):
            for cb, (a, b) in acc.items():
                acc_s[cb] = a
                acc_m[cb] = b

        def blocks(g, qm):
            out = []
            for ph in range(NPH):
                if isinstance(qm, int):
                    out.append(g * RS + (ph - qm) % NPH)
                else:
                    s = ph - qm
                    out.append(g * RS + jnp.where(s < 0, s + NPH, s))
            return out

        def super_step(g, q, qm, issue, last=False):
            blk = blocks(g, qm)
            i0 = g * RJ + q * SUB
            acc = {}
            for c in range(SUB):
                if issue and order == 'iw':
                    rd_start(i0 + c + depth)
                rd_wait(i0 + c)
                if issue and order == 'wi':
                    rd_start(i0 + c + depth)
                if mode == 'chunk':
                    if last and c == SUB - 1:
                        acc = {}
                    reduce_col(blk, q * SUB + c, c, acc)
                    if not (last and c == SUB - 1):
                        flush(acc)
                        acc = {}
            if mode == 'super':
                for c in range(SUB):
                    reduce_col(blk, q * SUB + c, c, acc)
                if not last:
                    flush(acc)
            return acc

        ntail = depth // SUB
        for g in range(NG):
            def body(q, qm, g=g):
                super_step(g, q, qm, True)
                return jnp.where(qm == NPH - 1, 0, qm + 1)

            lax.fori_loop(0, PJ - (ntail if g == NG - 1 else 0), body, jnp.int32(0))
            if g == 0:
                w1_cp.wait()
                w2_cp.wait()
                w1d[...] = dup_t(w1t_v)
            if g == 1:
                w2d[...] = dup_t(w2_v)
        for q in range(PJ - ntail, PJ):
            acc = super_step(NG - 1, q, q % NPH, False, last=(q == PJ - 1))

        lane = lax.broadcasted_iota(jnp.int32, (8, L), 1)
        hp = None
        for cb in range(CB):
            a, b = acc[cb] if cb in acc else (acc_s[cb], acc_m[cb])
            gap = jnp.sum(a, axis=1, keepdims=True) * (1.0 / (H * W))
            gmp = jnp.max(b, axis=1, keepdims=True)
            t = w1d[cb] * jnp.where(lane < 64, gap, gmp)
            hp = t if hp is None else hp + t

        for sh in (4, 2, 1):
            hp = hp + pltpu.roll(hp, sh, 0)
        hp = jnp.maximum(hp, 0.0)
        z = jnp.sum(w2d[...] * hp[None], axis=2, keepdims=True)
        sc = 0.5 * jnp.tanh(0.5 * z) + 0.5
        if rnd:
            sc = sc.astype(jnp.bfloat16).astype(jnp.float32)
        sc = jnp.broadcast_to(sc, (CB, 8, L))

        bufw = buf.reshape(PA, PJ, PR, L)

        def scale_piece(a, j, sq):
            v = bufw[a, j].astype(jnp.float32).reshape(TPP, 8, L)
            bufw[a, j] = (v * sq).reshape(PR, L).astype(jnp.bfloat16)

        def static_tab(p0):
            return jnp.stack([sc[((p0 + k) % PER) // WB] for k in range(TPP)], axis=0)

        def wr(a0, n, j):
            pltpu.make_async_copy(bufw.at[pl.ds(a0, n), j], o_hbm.at[pl.ds(a0, n), j], wsem).start()

        for j in range(peel):
            for s in range(NS):
                scale_piece(s, j, static_tab(TPP * (s + j)))
                if j == 0 and s == 0 and split1:
                    wr(0, 1, 0)
            if j == 0 and split1:
                wr(1, NS - 1, 0)
            else:
                wr(0, NS, j)

        for k in range(TAB):
            tab[k] = sc[k % CB]

        def wr_body(i, t):
            gq = lax.shift_right_logical(i, 6)
            j = i & (PJ - 1)
            a0 = gq * NS
            base = [lax.shift_right_logical((t + r) * 43, 7) for r in range(WB)]
            for s in range(NS):
                sq = jnp.stack([tab[base[(s * TPP + k) % WB] + (s * TPP + k) // WB] for k in range(TPP)], axis=0)
                scale_piece(a0 + s, j, sq)
            wr(a0, NS, j)
            t = t + jnp.where(j == PJ - 1, (NS - PJ + 1) * TPP % PER, TPP)
            return jnp.where(t >= PER, t - PER, t)

        lax.fori_loop(peel, (PA // NS) * PJ, wr_body, jnp.int32(peel * TPP % PER))
        pltpu.make_async_copy(bufw, o_hbm, wsem).wait()

    @jax.jit
    def fn(x, w1, w2):
        xv = jnp.transpose(x, (0, 1, 3, 2)).reshape(H, CB, 8, WB, L)
        xv = jnp.transpose(xv, (0, 1, 3, 2, 4)).reshape(PA, RJ, 16, L)
        out = pl.pallas_call(
            kernel,
            out_shape=jax.ShapeDtypeStruct((PA, PJ, PR, L), x.dtype),
            in_specs=[pl.BlockSpec(memory_space=pl.ANY)] * 3,
            out_specs=pl.BlockSpec(memory_space=pl.ANY),
            scratch_shapes=[
                pltpu.VMEM((PA, RJ, 16, L), jnp.bfloat16),
                pltpu.VMEM((R, C), jnp.bfloat16),
                pltpu.VMEM((R, C), jnp.bfloat16),
                pltpu.VMEM((CB, 8, L), jnp.float32),
                pltpu.VMEM((CB, 8, L), jnp.float32),
                pltpu.VMEM((CB, 8, L), jnp.float32),
                pltpu.VMEM((CB, 8, L), jnp.float32),
                pltpu.VMEM((TAB, 8, L), jnp.float32),
                pltpu.SemaphoreType.DMA((nsem,)),
                pltpu.SemaphoreType.DMA(()),
            ],
            compiler_params=pltpu.CompilerParams(vmem_limit_bytes=100 * 1024 * 1024,
                                                 disable_bounds_checks=True,
                                                 disable_semaphore_checks=True),
            name=name,
        )(xv, w1.T, w2)
        out = out.reshape(H, CB, WB, 8, L)
        out = jnp.transpose(out, (0, 1, 3, 2, 4)).reshape(1, H, C, W)
        return jnp.transpose(out, (0, 1, 3, 2))
    return fn

_impl = make_kernel(name='cbam_channel_attn')


@jax.jit
def pallas_standalone__channel_attn_cbam__vision_kernel(x, w1, w2):
    return _impl(x, w1, w2)
```

```python
import jax
import jax.numpy as jnp
from jax import lax
import jax.experimental.pallas as pl
import jax.experimental.pallas.tpu as pltpu

_H, _W, _C, _R = 384, 384, 192, 48
_L = 128
_WB = _W // _L
_CB = _C // 8
_PER = _CB * _WB

_NBLK = 54
_PJ, _PR = 64, 64
_TPP = _PR // 8
_NPH = _PER // _TPP
_WS = 6
_WSPLIT = (1, 2, 3)
_TAB = (_PER - _TPP + _WS * _TPP + 2) // _WB + 1
_RJ = 256
_SUB = _RJ // _PJ
_RS = 2 * _NPH
_NG = _NBLK // _RS
_NCH = _NG * _RJ
_N0 = 4
_D0, _D1 = 8, 16
_NSEM = 32


def _kernel(x_hbm, w1t_hbm, w2_hbm, o_hbm, buf, w1t_v, w2_v, w1d, w2d,
            acc_s, acc_m, tab, sems, wsem):
    bufw = buf.reshape(_NBLK, _PJ, _PR, _L)

    def chunk_copy(n, first, count):
        if isinstance(n, int):
            g, j, k = n // _RJ, n % _RJ, n % _NSEM
        else:
            g, j, k = lax.shift_right_logical(n, 8), n & (_RJ - 1), n & (_NSEM - 1)
        sl = (pl.ds(g * _RS + first, count), j)
        return pltpu.make_async_copy(x_hbm.at[sl], buf.at[sl], sems.at[k])

    def start(n, prio):
        if isinstance(n, int) and n >= _NCH:
            return
        first, count = (0, _N0) if prio == 0 else (_N0, _RS - _N0)
        chunk_copy(n, first, count).start(priority=prio)

    def step(n):
        chunk_copy(n, 0, _RS).wait()
        start(n + _D0, 0)
        start(n + _D1, 1)

    w1_cp = pltpu.make_async_copy(w1t_hbm, w1t_v, wsem)
    w2_cp = pltpu.make_async_copy(w2_hbm, w2_v, wsem)
    for n in range(_D1):
        start(n, 1)
        if n < _D0:
            start(n, 0)
    w1_cp.start()
    w2_cp.start()

    acc_s[...] = jnp.zeros(acc_s.shape, jnp.float32)
    acc_m[...] = jnp.full(acc_m.shape, -jnp.inf, jnp.float32)

    def dup_t(w_ref, s0, s1):
        w = w_ref[...].astype(jnp.float32)
        pad = jnp.zeros((_L // 2 - _R, _C), jnp.float32)
        return jnp.concatenate([w * s0, pad, w * s1, pad], axis=0).T.reshape(_CB, 8, _L)

    def reduce_column(blk, j, c):
        acc = {}
        for ph in range(_NPH):
            u = buf[blk[ph], j].astype(jnp.float32)
            v = buf[blk[ph] + _NPH, j].astype(jnp.float32)
            s = u + v
            m = jnp.maximum(u, v)
            for half in range(2):
                cb = (ph * _TPP + 2 * c + half) // _WB
                a, b = acc[cb] if cb in acc else (acc_s[cb], acc_m[cb])
                rows = slice(half * 8, half * 8 + 8)
                acc[cb] = (a + s[rows], jnp.maximum(b, m[rows]))
        return acc

    def flush(acc):
        for cb, (a, b) in acc.items():
            acc_s[cb] = a
            acc_m[cb] = b

    n_static = -(-_D1 // _SUB)
    for g in range(_NG):
        def body(q, qm, g=g):
            blk = [g * _RS + jnp.where(ph < qm, ph - qm + _NPH, ph - qm)
                   for ph in range(_NPH)]
            for c in range(_SUB):
                step(g * _RJ + q * _SUB + c)
                flush(reduce_column(blk, q * _SUB + c, c))
            return jnp.where(qm == _NPH - 1, 0, qm + 1)

        lax.fori_loop(0, _PJ - (n_static if g == _NG - 1 else 0), body, jnp.int32(0))
        if g == 0:
            w1_cp.wait()
            w2_cp.wait()
            w1d[...] = dup_t(w1t_v, 1.0 / (_H * _W), 1.0)
        if g == 1:
            w2d[...] = dup_t(w2_v, 0.5, 0.5)
    for n in range(_NCH - n_static * _SUB, _NCH):
        j = n % _RJ
        q, c = divmod(j, _SUB)
        step(n)
        acc = reduce_column(
            [(_NG - 1) * _RS + (ph - q) % _NPH for ph in range(_NPH)], j, c)
        if n < _NCH - 1:
            flush(acc)

    lane = lax.broadcasted_iota(jnp.int32, (8, _L), 1)
    hid = None
    for cb in sorted(range(_CB), key=lambda cb: cb in acc):
        a, b = acc[cb] if cb in acc else (acc_s[cb], acc_m[cb])
        pooled = jnp.where(lane < _L // 2,
                           jnp.sum(a, axis=1, keepdims=True),
                           jnp.max(b, axis=1, keepdims=True))
        t = w1d[cb] * pooled
        hid = t if hid is None else hid + t
    for shift in (4, 2, 1):
        hid = hid + pltpu.roll(hid, shift, 0)
    hid = jnp.maximum(hid, 0.0)
    z_half = jnp.sum(w2d[...] * hid[None], axis=2, keepdims=True)
    scale = 0.5 * jnp.tanh(z_half) + 0.5
    scale = scale.astype(jnp.bfloat16).astype(jnp.float32)
    scale = jnp.broadcast_to(scale, (_CB, 8, _L))

    def scale_piece(a, j, tile_scales):
        v = bufw[a, j].astype(jnp.float32).reshape(_TPP, 8, _L)
        v = v * jnp.stack(tile_scales, axis=0)
        bufw[a, j] = v.reshape(_PR, _L).astype(jnp.bfloat16)

    def write(a0, count, j):
        sl = (pl.ds(a0, count), j)
        pltpu.make_async_copy(bufw.at[sl], o_hbm.at[sl], wsem).start()

    a0 = 0
    for count in _WSPLIT:
        for a in range(a0, a0 + count):
            scale_piece(a, 0, [scale[(a * _TPP + k) // _WB] for k in range(_TPP)])
        write(a0, count, 0)
        a0 += count

    for k in range(_TAB):
        tab[k] = scale[k % _CB]

    def write_body(i, t):
        a0 = lax.shift_right_logical(i, 6) * _WS
        j = i & (_PJ - 1)
        base = [lax.shift_right_logical((t + r) * 43, 7) for r in range(_WB)]
        for s in range(_WS):
            ks = range(s * _TPP, (s + 1) * _TPP)
            scale_piece(a0 + s, j, [tab[base[k % _WB] + k // _WB] for k in ks])
        write(a0, _WS, j)
        t = t + jnp.where(j == _PJ - 1, (_WS - _PJ + 1) * _TPP % _PER, _TPP)
        return jnp.where(t >= _PER, t - _PER, t)

    lax.fori_loop(1, (_NBLK // _WS) * _PJ, write_body, jnp.int32(_TPP))
    pltpu.make_async_copy(bufw, o_hbm, wsem).wait()


@jax.jit
def pallas_standalone__channel_attn_cbam__vision_kernel(
    x: jax.Array,
    w1: jax.Array,
    w2: jax.Array,
):
    assert x.shape == (1, _H, _W, _C) and w1.shape == (_C, _R) and w2.shape == (_R, _C)
    xv = jnp.transpose(x, (0, 1, 3, 2)).reshape(_H, _CB, 8, _WB, _L)
    xv = jnp.transpose(xv, (0, 1, 3, 2, 4)).reshape(_NBLK, _RJ, 16, _L)
    vec = pltpu.VMEM((_CB, 8, _L), jnp.float32)
    out = pl.pallas_call(
        _kernel,
        out_shape=jax.ShapeDtypeStruct((_NBLK, _PJ, _PR, _L), x.dtype),
        in_specs=[pl.BlockSpec(memory_space=pl.ANY)] * 3,
        out_specs=pl.BlockSpec(memory_space=pl.ANY),
        scratch_shapes=[
            pltpu.VMEM((_NBLK, _RJ, 16, _L), x.dtype),
            pltpu.VMEM((_R, _C), w1.dtype),
            pltpu.VMEM((_R, _C), w2.dtype),
            vec, vec,
            vec, vec,
            pltpu.VMEM((_TAB, 8, _L), jnp.float32),
            pltpu.SemaphoreType.DMA((_NSEM,)),
            pltpu.SemaphoreType.DMA(()),
        ],
        compiler_params=pltpu.CompilerParams(
            vmem_limit_bytes=100 * 1024 * 1024,
            disable_bounds_checks=True,
            disable_semaphore_checks=True,
        ),
        name="cbam_channel_attn",
    )(xv, w1.T, w2)
    out = out.reshape(_H, _CB, _WB, 8, _L)
    out = jnp.transpose(out, (0, 1, 3, 2, 4)).reshape(1, _H, _C, _W)
    return jnp.transpose(out, (0, 1, 3, 2))
```

```python
import jax
import jax.numpy as jnp
from jax import lax
import jax.experimental.pallas as pl
import jax.experimental.pallas.tpu as pltpu

_H, _W, _C, _R = 384, 384, 192, 48
_L = 128
_WB = _W // _L
_CB = _C // 8
_PER = _CB * _WB

_NBLK, _PJ, _SUB = 54, 64, 4
_VIEW = (_NBLK, _PJ, _SUB, 16, _L)
_TPP = 2 * _SUB
_NPH = _PER // _TPP
_RS = 2 * _NPH
_NG = _NBLK // _RS
_N0 = 4
_D0, _D1 = 2, 4
_RING = 8
_WS = 6
_WSPLIT = (1, 2, 3)
_TAB = (_PER - _TPP + _WS * _TPP + 2) // _WB + 1


def _kernel(x_hbm, w1t_hbm, w2_hbm, o_hbm, buf, w1t_v, w2_v, w1d, w2d,
            acc_s, acc_m, tab, sems, wsem):
    def chunk_copy(p, c, first, count):
        if isinstance(p, int):
            g, q, k = p // _PJ, p % _PJ, p % _RING
        else:
            g, q, k = lax.shift_right_logical(p, 6), p & (_PJ - 1), p & (_RING - 1)
        sl = (pl.ds(g * _RS + first, count), q, c)
        return pltpu.make_async_copy(x_hbm.at[sl], buf.at[sl], sems.at[k * _SUB + c])

    def start(p, c, prio):
        if isinstance(p, int) and p >= _NG * _PJ:
            return
        first, count = (0, _N0) if prio == 0 else (_N0, _RS - _N0)
        chunk_copy(p, c, first, count).start(priority=prio)

    def step(p, c):
        chunk_copy(p, c, 0, _RS).wait()
        start(p + _D0, c, 0)
        start(p + _D1, c, 1)

    w1_cp = pltpu.make_async_copy(w1t_hbm, w1t_v, wsem)
    w2_cp = pltpu.make_async_copy(w2_hbm, w2_v, wsem)
    for p in range(_D1):
        for c in range(_SUB):
            start(p, c, 1)
            if p < _D0:
                start(p, c, 0)
    w1_cp.start()
    w2_cp.start()

    acc_s[...] = jnp.zeros(acc_s.shape, jnp.float32)
    acc_m[...] = jnp.full(acc_m.shape, -jnp.inf, jnp.float32)

    def dup_t(w_ref, s0, s1):
        w = w_ref[...].astype(jnp.float32)
        pad = jnp.zeros((_L // 2 - _R, _C), jnp.float32)
        return jnp.concatenate([w * s0, pad, w * s1, pad], axis=0).T.reshape(_CB, 8, _L)

    def reduce_column(blk, q, c):
        acc = {}
        for ph in range(_NPH):
            u = buf[blk[ph], q, c].astype(jnp.float32)
            v = buf[blk[ph] + _NPH, q, c].astype(jnp.float32)
            s = u + v
            m = jnp.maximum(u, v)
            for half in range(2):
                cb = (ph * _TPP + 2 * c + half) // _WB
                a, b = acc[cb] if cb in acc else (acc_s[cb], acc_m[cb])
                rows = slice(half * 8, half * 8 + 8)
                acc[cb] = (a + s[rows], jnp.maximum(b, m[rows]))
        return acc

    def flush(acc):
        for cb, (a, b) in acc.items():
            acc_s[cb] = a
            acc_m[cb] = b

    for g in range(_NG):
        def body(q, qm, g=g):
            blk = [g * _RS + jnp.where(ph < qm, ph - qm + _NPH, ph - qm)
                   for ph in range(_NPH)]
            for c in range(_SUB):
                step(g * _PJ + q, c)
                flush(reduce_column(blk, q, c))
            return jnp.where(qm == _NPH - 1, 0, qm + 1)

        lax.fori_loop(0, _PJ - (_D1 if g == _NG - 1 else 0), body, jnp.int32(0))
        if g == 0:
            w1_cp.wait()
            w2_cp.wait()
            w1d[...] = dup_t(w1t_v, 1.0 / (_H * _W), 1.0)
        if g == 1:
            w2d[...] = dup_t(w2_v, 0.5, 0.5)
    for q in range(_PJ - _D1, _PJ):
        blk = [(_NG - 1) * _RS + (ph - q) % _NPH for ph in range(_NPH)]
        for c in range(_SUB):
            step((_NG - 1) * _PJ + q, c)
            acc = reduce_column(blk, q, c)
            if (q, c) != (_PJ - 1, _SUB - 1):
                flush(acc)

    lane = lax.broadcasted_iota(jnp.int32, (8, _L), 1)
    hid = None
    for cb in sorted(range(_CB), key=lambda cb: cb in acc):
        a, b = acc[cb] if cb in acc else (acc_s[cb], acc_m[cb])
        pooled = jnp.where(lane < _L // 2,
                           jnp.sum(a, axis=1, keepdims=True),
                           jnp.max(b, axis=1, keepdims=True))
        t = w1d[cb] * pooled
        hid = t if hid is None else hid + t
    for shift in (4, 2, 1):
        hid = hid + pltpu.roll(hid, shift, 0)
    hid = jnp.maximum(hid, 0.0)
    z_half = jnp.sum(w2d[...] * hid[None], axis=2, keepdims=True)
    scale = 0.5 * jnp.tanh(z_half) + 0.5
    scale = scale.astype(jnp.bfloat16).astype(jnp.float32)
    scale = jnp.broadcast_to(scale, (_CB, 8, _L))

    def scale_piece(a, j, tile_scales):
        v = buf[a, j].astype(jnp.float32).reshape(_TPP, 8, _L)
        v = v * jnp.stack(tile_scales, axis=0)
        buf[a, j] = v.reshape(_SUB, 16, _L).astype(jnp.bfloat16)

    def write(a0, count, j):
        sl = (pl.ds(a0, count), j)
        pltpu.make_async_copy(buf.at[sl], o_hbm.at[sl], wsem).start()

    a0 = 0
    for count in _WSPLIT:
        for a in range(a0, a0 + count):
            scale_piece(a, 0, [scale[(a * _TPP + k) // _WB] for k in range(_TPP)])
        write(a0, count, 0)
        a0 += count

    for k in range(_TAB):
        tab[k] = scale[k % _CB]

    def write_body(i, t):
        a0 = lax.shift_right_logical(i, 6) * _WS
        j = i & (_PJ - 1)
        base = [lax.shift_right_logical((t + r) * 43, 7) for r in range(_WB)]
        for s in range(_WS):
            ks = range(s * _TPP, (s + 1) * _TPP)
            scale_piece(a0 + s, j, [tab[base[k % _WB] + k // _WB] for k in ks])
        write(a0, _WS, j)
        t = t + jnp.where(j == _PJ - 1, (_WS - _PJ + 1) * _TPP % _PER, _TPP)
        return jnp.where(t >= _PER, t - _PER, t)

    lax.fori_loop(1, (_NBLK // _WS) * _PJ, write_body, jnp.int32(_TPP))
    pltpu.make_async_copy(buf, o_hbm, wsem).wait()


@jax.jit
def pallas_standalone__channel_attn_cbam__vision_kernel(
    x: jax.Array,
    w1: jax.Array,
    w2: jax.Array,
):
    assert x.shape == (1, _H, _W, _C) and w1.shape == (_C, _R) and w2.shape == (_R, _C)
    xv = jnp.transpose(x, (0, 1, 3, 2)).reshape(_H, _CB, 8, _WB, _L)
    xv = jnp.transpose(xv, (0, 1, 3, 2, 4)).reshape(_VIEW)
    vec = pltpu.VMEM((_CB, 8, _L), jnp.float32)
    out = pl.pallas_call(
        _kernel,
        out_shape=jax.ShapeDtypeStruct(_VIEW, x.dtype),
        in_specs=[pl.BlockSpec(memory_space=pl.ANY)] * 3,
        out_specs=pl.BlockSpec(memory_space=pl.ANY),
        scratch_shapes=[
            pltpu.VMEM(_VIEW, x.dtype),
            pltpu.VMEM((_R, _C), w1.dtype),
            pltpu.VMEM((_R, _C), w2.dtype),
            vec, vec,
            vec, vec,
            pltpu.VMEM((_TAB, 8, _L), jnp.float32),
            pltpu.SemaphoreType.DMA((_RING * _SUB,)),
            pltpu.SemaphoreType.DMA(()),
        ],
        compiler_params=pltpu.CompilerParams(
            vmem_limit_bytes=100 * 1024 * 1024,
            disable_bounds_checks=True,
            disable_semaphore_checks=True,
        ),
        name="cbam_channel_attn",
    )(xv, w1.T, w2)
    out = out.reshape(_H, _CB, _WB, 8, _L)
    out = jnp.transpose(out, (0, 1, 3, 2, 4)).reshape(1, _H, _C, _W)
    return jnp.transpose(out, (0, 1, 3, 2))
```

```python
import jax
import jax.numpy as jnp
from jax import lax
import jax.experimental.pallas as pl
import jax.experimental.pallas.tpu as pltpu

_H, _W, _C, _R = 384, 384, 192, 48
_L = 128
_WB = _W // _L
_CB = _C // 8
_PER = _CB * _WB

_NBLK, _PJ, _SUB = 54, 64, 4
_VIEW = (_NBLK, _PJ, _SUB, 16, _L)
_TPP = 2 * _SUB
_NPH = _PER // _TPP
_RS = 2 * _NPH
_NG = _NBLK // _RS
_N0 = 4
_D0, _D1 = 2, 4
_RING = _D1
_WS = 6
_WSPLIT = (1, 2, 3)
_TAB = (_PER - _TPP + _WS * _TPP + 2) // _WB + 1


def _kernel(x_hbm, w1t_hbm, w2_hbm, o_hbm, buf, w1t_v, w2_v, w1d, w2d,
            acc_s, acc_m, tab, sems, wsem):
    def chunk_copy(p, c, first, count):
        if isinstance(p, int):
            g, q, k = p // _PJ, p % _PJ, p % _RING
        else:
            g, q, k = lax.shift_right_logical(p, 6), p & (_PJ - 1), p & (_RING - 1)
        sl = (pl.ds(g * _RS + first, count), q, c)
        return pltpu.make_async_copy(x_hbm.at[sl], buf.at[sl], sems.at[k * _SUB + c])

    def start(p, c, prio):
        if isinstance(p, int) and p >= _NG * _PJ:
            return
        first, count = (0, _N0) if prio == 0 else (_N0, _RS - _N0)
        chunk_copy(p, c, first, count).start(priority=prio)

    def step(p, c):
        chunk_copy(p, c, 0, _RS).wait()
        start(p + _D0, c, 0)
        start(p + _D1, c, 1)

    def init_rows(ref, value, lo, hi):
        def body(cb, carry):
            ref[cb] = jnp.full((8, _L), value, jnp.float32)
            return carry

        lax.fori_loop(lo, hi, body, 0)

    head = [(p, c) for p in range(_D1) for c in range(_SUB)]
    start(0, 0, 1)
    start(0, 0, 0)
    for p, c in head[1:]:
        start(p, c, 1)
    fill = ([(acc_s, 0.0, lo, lo + 8) for lo in range(0, _CB, 8)]
            + [(acc_m, -jnp.inf, lo, lo + 6) for lo in range(0, _CB, 6)])
    for (p, c), rows in zip(head[1:_D0 * _SUB], fill, strict=True):
        init_rows(*rows)
        start(p, c, 0)
    w1_cp = pltpu.make_async_copy(w1t_hbm, w1t_v, wsem)
    w2_cp = pltpu.make_async_copy(w2_hbm, w2_v, wsem)
    w1_cp.start(priority=1)
    w2_cp.start(priority=1)

    def dup_t(w_ref, s0, s1):
        w = w_ref[...].astype(jnp.float32)
        pad = jnp.zeros((_L // 2 - _R, _C), jnp.float32)
        return jnp.concatenate([w * s0, pad, w * s1, pad], axis=0).T.reshape(_CB, 8, _L)

    def reduce_column(blk, q, c):
        acc = {}
        for ph in range(_NPH):
            u = buf[blk[ph], q, c].astype(jnp.float32)
            v = buf[blk[ph] + _NPH, q, c].astype(jnp.float32)
            s = u + v
            m = jnp.maximum(u, v)
            for half in range(2):
                cb = (ph * _TPP + 2 * c + half) // _WB
                a, b = acc[cb] if cb in acc else (acc_s[cb], acc_m[cb])
                rows = slice(half * 8, half * 8 + 8)
                acc[cb] = (a + s[rows], jnp.maximum(b, m[rows]))
        return acc

    def flush(acc):
        for cb, (a, b) in acc.items():
            acc_s[cb] = a
            acc_m[cb] = b

    for g in range(_NG):
        def body(q, qm, g=g):
            blk = [g * _RS + jnp.where(ph < qm, ph - qm + _NPH, ph - qm)
                   for ph in range(_NPH)]
            for c in range(_SUB):
                step(g * _PJ + q, c)
                flush(reduce_column(blk, q, c))
            return jnp.where(qm == _NPH - 1, 0, qm + 1)

        lax.fori_loop(0, _PJ - (_D1 if g == _NG - 1 else 0), body, jnp.int32(0))
        if g == 0:
            w1_cp.wait()
            w2_cp.wait()
            w1d[...] = dup_t(w1t_v, 1.0 / (_H * _W), 1.0)
        if g == 1:
            w2d[...] = dup_t(w2_v, 0.5, 0.5)
    for q in range(_PJ - _D1, _PJ):
        blk = [(_NG - 1) * _RS + (ph - q) % _NPH for ph in range(_NPH)]
        for c in range(_SUB):
            step((_NG - 1) * _PJ + q, c)
            acc = reduce_column(blk, q, c)
            if (q, c) != (_PJ - 1, _SUB - 1):
                flush(acc)

    lane = lax.broadcasted_iota(jnp.int32, (8, _L), 1)
    hid = None
    for cb in sorted(range(_CB), key=lambda cb: cb in acc):
        a, b = acc[cb] if cb in acc else (acc_s[cb], acc_m[cb])
        pooled = jnp.where(lane < _L // 2,
                           jnp.sum(a, axis=1, keepdims=True),
                           jnp.max(b, axis=1, keepdims=True))
        t = w1d[cb] * pooled
        hid = t if hid is None else hid + t
    for shift in (4, 2, 1):
        hid = hid + pltpu.roll(hid, shift, 0)
    hid = jnp.maximum(hid, 0.0)
    z_half = jnp.sum(w2d[...] * hid[None], axis=2, keepdims=True)
    scale = 0.5 * jnp.tanh(z_half) + 0.5
    scale = scale.astype(jnp.bfloat16).astype(jnp.float32)
    scale = jnp.broadcast_to(scale, (_CB, 8, _L))

    def scale_piece(a, j, tile_scales):
        v = buf[a, j].astype(jnp.float32).reshape(_TPP, 8, _L)
        v = v * jnp.stack(tile_scales, axis=0)
        buf[a, j] = v.reshape(_SUB, 16, _L).astype(jnp.bfloat16)

    def write(*sl):
        pltpu.make_async_copy(buf.at[sl], o_hbm.at[sl], wsem).start()

    a0 = 0
    for count in _WSPLIT:
        for a in range(a0, a0 + count):
            scale_piece(a, 0, [scale[(a * _TPP + k) // _WB] for k in range(_TPP)])
        write(pl.ds(a0, count), 0)
        a0 += count

    for k in range(_TAB):
        tab[k] = scale[k % _CB]

    def write_body(i, t):
        a0 = lax.shift_right_logical(i, 6) * _WS
        j = i & (_PJ - 1)
        base = [lax.shift_right_logical((t + r) * 43, 7) for r in range(_WB)]
        for s in range(_WS):
            ks = range(s * _TPP, (s + 1) * _TPP)
            scale_piece(a0 + s, j, [tab[base[k % _WB] + k // _WB] for k in ks])
        for c in range(_SUB):
            write(pl.ds(a0, _WS), j, c)
        t = t + jnp.where(j == _PJ - 1, (_WS - _PJ + 1) * _TPP % _PER, _TPP)
        return jnp.where(t >= _PER, t - _PER, t)

    lax.fori_loop(1, (_NBLK // _WS) * _PJ, write_body, jnp.int32(_TPP))
    pltpu.make_async_copy(buf, o_hbm, wsem).wait()


@jax.jit
def pallas_standalone__channel_attn_cbam__vision_kernel(
    x: jax.Array,
    w1: jax.Array,
    w2: jax.Array,
):
    assert x.shape == (1, _H, _W, _C) and w1.shape == (_C, _R) and w2.shape == (_R, _C)
    xv = jnp.transpose(x, (0, 1, 3, 2)).reshape(_H, _CB, 8, _WB, _L)
    xv = jnp.transpose(xv, (0, 1, 3, 2, 4)).reshape(_VIEW)
    vec = pltpu.VMEM((_CB, 8, _L), jnp.float32)
    out = pl.pallas_call(
        _kernel,
        out_shape=jax.ShapeDtypeStruct(_VIEW, x.dtype),
        in_specs=[pl.BlockSpec(memory_space=pl.ANY)] * 3,
        out_specs=pl.BlockSpec(memory_space=pl.ANY),
        scratch_shapes=[
            pltpu.VMEM(_VIEW, x.dtype),
            pltpu.VMEM((_R, _C), w1.dtype),
            pltpu.VMEM((_R, _C), w2.dtype),
            vec, vec,
            vec, vec,
            pltpu.VMEM((_TAB, 8, _L), jnp.float32),
            pltpu.SemaphoreType.DMA((_RING * _SUB,)),
            pltpu.SemaphoreType.DMA(()),
        ],
        compiler_params=pltpu.CompilerParams(
            vmem_limit_bytes=100 * 1024 * 1024,
            disable_bounds_checks=True,
            disable_semaphore_checks=True,
        ),
        name="cbam_channel_attn",
    )(xv, w1.T, w2)
    out = out.reshape(_H, _CB, _WB, 8, _L)
    out = jnp.transpose(out, (0, 1, 3, 2, 4)).reshape(1, _H, _C, _W)
    return jnp.transpose(out, (0, 1, 3, 2))
```
